```python
import os as _os
_os.environ.setdefault("JAX_PLATFORMS", "cpu")
import jax
import jax.numpy as jnp

def _softmax(x, axis=-1):
    return jax.nn.softmax(x, axis=axis)
def _gelu(x):
    return jax.nn.gelu(x, approximate=True)
def _silu(x):
    return jax.nn.silu(x)
def _sigmoid(x):
    return jax.nn.sigmoid(x)
def _layernorm(x, axis=-1, eps=1e-5):
    m = jnp.mean(x, axis=axis, keepdims=True)
    v = jnp.var(x, axis=axis, keepdims=True)
    return (x - m) / jnp.sqrt(v + eps)
def _scatter_add(tgt, idx, src, axis=0):
    return tgt.at[idx].add(src)
def _segment_sum(src, seg, n):
    return jax.ops.segment_sum(src, seg, n)
class _Rng:
    def __init__(self, key):
        self._k = key
    def _next(self):
        self._k, sub = jax.random.split(self._k)
        return sub
    def normal(self, shape):
        return jax.random.normal(self._next(), shape, dtype=jnp.bfloat16)
    def randint(self, lo, hi, shape):
        return jax.random.randint(self._next(), shape, lo, hi, dtype=jnp.int32)
    def uniform(self, shape, lo=0.0, hi=1.0):
        return jax.random.uniform(self._next(), shape, jnp.bfloat16, lo, hi)
    def permutation(self, n):
        return jax.random.permutation(self._next(), n)


kernel_name = 'gated_mix__sliding_block__dense_activation_silu__prompt'

def setup_inputs():
    _rng = _Rng(jax.random.key(int.from_bytes(__import__("os").urandom(4), "little")))
    _w = (lambda a: (lambda t: t.astype(jnp.bfloat16) if jnp.issubdtype(t.dtype, jnp.floating) else t)(jnp.asarray(a)))
    def _A_setup():
        B, S, D = 1, 2048, 640
        return {
            "x": _w((lambda *s: _rng.normal(s) * 0.05)(B, S, D)),
            "wqkv": _w((lambda *s: _rng.normal(s) * 0.4)(D, 3 * D)),
            "wo": _w((lambda *s: _rng.normal(s) * 0.05)(D, D)),
        }
    _A_in = _A_setup()

    def _B_setup():
        B, S, D, F = 1, 2048, 640, 1536
        return {
            "x": _w((lambda *s: _rng.normal(s) * 0.05)(B, S, D)),
            "w1": _w((lambda *s: _rng.normal(s) * 1.6)(D, F) * (D ** -0.5)),
            "w2": _w((lambda *s: _rng.normal(s) * 1.6)(F, D) * (F ** -0.5)),
        }
    _B_in = _B_setup()

    return {
        "A_x": _A_in["x"],
        "A_wqkv": _A_in["wqkv"],
        "A_wo": _A_in["wo"],
        "B_x": _B_in["x"],
        "B_w1": _B_in["w1"],
        "B_w2": _B_in["w2"],
        "gate_w": _w((lambda *s: _rng.normal(s) * 0.05)(640) * 16.0),
    }

def reference(A_x, A_wqkv, A_wo, B_x, B_w1, B_w2, gate_w):
    def _A_ref(x, wqkv, wo):
        B, S, D = x.shape
        H = 32; Dh = D // H; W = 256
        qkv = (lambda x, *d: x.transpose(*d))((x @ wqkv).reshape(B, S, 3, H, Dh), 2, 0, 3, 1, 4)
        q, k, v = qkv[0], qkv[1], qkv[2]
        scores = jnp.einsum("bhqd,bhkd->bhqk", q, k) * (Dh ** -0.5)
        idx = jnp.arange(S)
        mask = (idx[:, None] - idx[None, :] >= 0) & (idx[:, None] - idx[None, :] < W)
        scores = jnp.where(mask[None, None], scores, -1e9)
        p = _softmax(scores, axis=-1)
        o = jnp.einsum("bhqk,bhkd->bhqd", p, v)
        return (lambda x, *d: x.transpose(*d))(o, 0, 2, 1, 3).reshape(B, S, D) @ wo

    def _B_ref(x, w1, w2):
        h = jnp.einsum("bsd,df->bsf", x, w1)
        h = _silu(h)
        out = jnp.einsum("bsf,fd->bsd", h, w2)
        return out

    x = A_x
    g = _sigmoid((x * gate_w).sum(-1, keepdims=True))
    a = _A_ref(x, A_wqkv, A_wo)
    b = _B_ref(x, B_w1, B_w2)
    return g * a + (1 - g) * b
```

```python
import functools
import math

import jax
import jax.numpy as jnp
import numpy as np
from jax import lax
import jax.experimental.pallas as pl
import jax.experimental.pallas.tpu as pltpu

S = 2048
D = 640
H = 32
DH = 20
F = 1536
QB = 128
NBLK = S // QB + 2
NG = 8
NEG = -1e30

OPT = dict(TM=512, LP=False, PACK=1, FSPLIT=0, GATE=0, SKEW=1, WOFIRST=1, KFIRST=0)

NT = (((1,), (1,)), ((), ()))


def group_window(g):
    return 64 * ((80 * g) // 64)


def flag_lane(g):
    return (80 * g + 80) % 128


def make_kernel(TM, LP, PACK, FSPLIT, GATE, SKEW, WOFIRST, KFIRST):
    NQ = TM // QB
    NS = S // TM
    f32, bf16, u32 = jnp.float32, jnp.bfloat16, jnp.uint32

    def ld(v):
        return pltpu.bitcast(v, bf16) if PACK else v

    def st(v):
        return pltpu.bitcast(v, u32) if PACK else v

    R = 2 if PACK else 1

    def kernel(x_hbm, wqkv_hbm, wo_hbm, w1_hbm, w2_hbm, gw_hbm, o_ref,
               kc_ref, vt_ref, q_ref, wvt_ref, co_ref, ch_ref, g_ref,
               xs_ref, wqk_ref, wv_ref, wo_ref, w1_ref, w2_ref, gw_ref, sems):
        i = pl.program_id(0)
        lane = lax.broadcasted_iota(jnp.int32, (QB // 2, 128), 1)

        def x_copy(c):
            return pltpu.make_async_copy(x_hbm.at[pl.ds(c * TM, TM)], xs_ref.at[c], sems.at[6 + c])
        wqk_copy = pltpu.make_async_copy(wqkv_hbm.at[:, pl.ds(0, 2 * D)], wqk_ref, sems.at[0])
        wv_copy = pltpu.make_async_copy(wqkv_hbm.at[:, pl.ds(2 * D, D)], wv_ref, sems.at[1])
        gw_copy = pltpu.make_async_copy(gw_hbm, gw_ref, sems.at[2])
        w1_copy = pltpu.make_async_copy(w1_hbm, w1_ref, sems.at[3])
        w2_copy = pltpu.make_async_copy(w2_hbm, w2_ref, sems.at[4])
        wo_copy = pltpu.make_async_copy(wo_hbm, wo_ref, sems.at[5])

        @pl.when(i == 0)
        def _():
            x_copy(0).start()
            gw_copy.start()
            wqk_copy.start()
            wv_copy.start()
            wo_copy.start()
            w1_copy.start()
            w2_copy.start()
            for c in range(1, NS):
                x_copy(c).start()
            lane_f = lax.broadcasted_iota(jnp.int32, (QB, 128), 1)
            for g in range(NG):
                pad = st(jnp.where(lane_f == flag_lane(g), NEG, 0.0).astype(bf16))
                kc_ref[0, g] = pad
                kc_ref[1, g] = pad
            vt_ref[0:2] = jnp.zeros((2, 768 // R, QB), vt_ref.dtype)
            gw_copy.wait()
            wqk_copy.wait()
            wv_copy.wait()
            for t in range(5):
                w = wv_ref[:, 128 * t: 128 * (t + 1)].astype(f32)
                wvt_ref[128 * t:128 * (t + 1), :] = w.T.astype(bf16)

        x_copy(i).wait()
        x = xs_ref[i]

        def head_mask(g, t):
            a = (DH * (4 * g + t)) % 128
            b = a + DH
            m = (lane >= a) & (lane < b)
            if b > 128:
                m = m | (lane < b - 128)
            return m | (lane == flag_lane(g))

        scale = (DH ** -0.5) * math.log2(math.e)
        if KFIRST:
            k = jnp.dot(x, wqk_ref[:, D:2 * D], preferred_element_type=f32).astype(bf16)
            q = (jnp.dot(x, wqk_ref[:, 0:D], preferred_element_type=f32) * scale).astype(bf16)
        else:
            qk = jnp.dot(x, wqk_ref[...], preferred_element_type=f32)
            q = (qk[:, 0:D] * scale).astype(bf16)
            k = qk[:, D:2 * D].astype(bf16)
        one2 = jnp.uint32(0x3F803F80)
        for j in range(NQ):
            blk = 2 + i * NQ + j
            for is_q, arr, flag in ((False, k, jnp.uint32(0)), (True, q, one2)):
                slabs = [pltpu.bitcast(arr[j * QB:(j + 1) * QB, 128 * t:128 * (t + 1)], u32) for t in range(5)]
                for g in range(NG):
                    w0 = group_window(g)
                    t = w0 // 128
                    if w0 % 128 == 0:
                        win = slabs[t]
                    else:
                        win = jnp.where(lane < 64, slabs[t + 1], slabs[t])
                    win = jnp.where(lane == flag_lane(g), flag, win)
                    win = win if PACK else pltpu.bitcast(win, bf16)
                    if not is_q:
                        kc_ref[blk, g] = win
                    else:
                        q_ref[j, g] = win

        vt = lax.dot_general(wvt_ref[...], x, NT, preferred_element_type=f32)
        ones = jnp.ones((8, TM), f32)
        parts = []
        for p in range(16):
            b = 40 * p
            parts += [vt[b:b + 24], ones, vt[b + 24:b + 40]]
        vtp = st(jnp.concatenate(parts, axis=0).astype(bf16))
        for j in range(NQ):
            vt_ref[2 + i * NQ + j] = vtp[:, j * QB:(j + 1) * QB]

        logit = jnp.sum(x.astype(f32) * gw_ref[...].astype(f32)[None, :], axis=1, keepdims=True)
        g_ = jax.nn.sigmoid(logit)
        g_ref[...] = jnp.broadcast_to(g_, (TM, 128))

        row = lax.broadcasted_iota(jnp.int32, (QB, QB), 0)
        col = lax.broadcasted_iota(jnp.int32, (QB, QB), 1)
        tri = row > col
        sub = lax.broadcasted_iota(jnp.int32, (8, QB), 0)

        def a_dot(j, jg, g):
            qw = q_ref[j, g] if PACK else pltpu.bitcast(q_ref[j, g], u32)
            qm = jnp.concatenate(
                [pltpu.bitcast(jnp.where(head_mask(g, t), qw, jnp.uint32(0)), bf16) for t in range(4)], axis=0)
            ks = jnp.concatenate([ld(kc_ref[jg + c, g]) for c in range(3)], axis=0)
            return lax.dot_general(ks, qm, NT, preferred_element_type=f32)

        def a_post(s, t):
            st_ = s[:, 128 * t:128 * (t + 1)]
            comb = jnp.where(tri, st_[0:QB], st_[2 * QB:])
            s1 = st_[QB:2 * QB]
            m = jnp.maximum(jnp.max(comb, axis=0, keepdims=True), jnp.max(s1, axis=0, keepdims=True))
            return (m, comb, s1)

        def b_head(jg, g, t, stt):
            m, comb, s1 = stt
            h = 4 * g + t
            pc = jnp.exp2(comb - m)
            p1 = jnp.exp2(s1 - m)
            p0 = jnp.where(tri, pc, 0.0)
            p2 = jnp.where(tri, 0.0, pc)
            p = jnp.concatenate([p0, p1, p2], axis=0).astype(bf16)
            pair = h // 2
            ra = (48 * pair + (0 if h % 2 == 0 else 32)) // R
            rb = (48 * pair + 16) // R
            n = 16 // R
            lhs = jnp.concatenate(
                [jnp.concatenate([ld(vt_ref[jg + c, ra:ra + n, :]), ld(vt_ref[jg + c, rb:rb + n, :])], axis=0)
                 for c in range(3)], axis=1)
            r = jnp.dot(lhs, p, preferred_element_type=f32)
            inv = 1.0 / r[24:32]
            return (r[0:8] * inv, r[8:16] * inv, r[16:24] * inv)

        def pair_rows(e, o):
            return [e[0], e[1], jnp.where(sub < 4, e[2], o[2]), o[0], o[1]]

        def finish_block(j, rows):
            ot = jnp.concatenate(rows, axis=0)
            gg = g_ref[j * QB:(j + 1) * QB, :]
            for t in range(5):
                o_t = ot[128 * t:128 * (t + 1)].T
                co_ref[j * QB // R:(j + 1) * QB // R, 128 * t:128 * (t + 1)] = st((o_t * gg).astype(bf16))

        units = [(j, i * NQ + j, g) for j in range(NQ) for g in range(NG)]
        n = len(units)
        pend = {}

        def issue(u):
            s = a_dot(*units[u])
            pend[u] = [a_post(s, t) for t in range(4)]

        for u in range(min(SKEW, n)):
            issue(u)
        rows = []
        for u in range(n):
            j, jg, g = units[u]
            if u + SKEW < n:
                issue(u + SKEW)
            sts = pend.pop(u)
            res = [b_head(jg, g, t, sts[t]) for t in range(4)]
            rows += pair_rows(res[0], res[1]) + pair_rows(res[2], res[3])
            if g == NG - 1:
                finish_block(j, rows)
                rows = []

        @pl.when(i == 0)
        def _():
            wo_copy.wait()
            w1_copy.wait()
            w2_copy.wait()

        out = None
        if WOFIRST:
            out = jnp.dot(ld(co_ref[...]), wo_ref[...], preferred_element_type=f32)
        g1 = 1.0 - g_ref[:, 0:1]
        nf = max(FSPLIT, 1)
        fc = F // nf
        for c in range(nf):
            hh = jnp.dot(x, w1_ref[:, c * fc:(c + 1) * fc], preferred_element_type=f32)
            u_ = 0.5 * hh
            hs = ((u_ + u_ * jnp.tanh(u_)) * g1).astype(bf16)
            if FSPLIT:
                d = jnp.dot(hs, w2_ref[c * fc:(c + 1) * fc, :], preferred_element_type=f32)
                out = d if out is None else out + d
            else:
                ch_ref[...] = st(hs)
        if not FSPLIT:
            d = jnp.dot(ld(ch_ref[...]), w2_ref[...], preferred_element_type=f32)
            out = d if out is None else out + d
        if not WOFIRST:
            out = out + jnp.dot(ld(co_ref[...]), wo_ref[...], preferred_element_type=f32)
        o_ref[...] = out.astype(o_ref.dtype)

    return kernel


@jax.jit
def pallas_gated_mix__sliding_block__dense_activation_silu__prompt_kernel(
    A_x, A_wqkv, A_wo, B_x, B_w1, B_w2, gate_w):
    TM = OPT["TM"]
    NQ = TM // QB
    R = 2 if OPT["PACK"] else 1
    pk = jnp.uint32 if OPT["PACK"] else jnp.bfloat16
    x = A_x.reshape(S, D)
    hbm = pl.BlockSpec(memory_space=pl.ANY)
    flags = {"XLA_TPU_FORCE_LP_LLO_SCHEDULER": True} if OPT["LP"] else None
    out = pl.pallas_call(
        make_kernel(**OPT),
        grid=(S // TM,),
        in_specs=[hbm] * 6,
        out_specs=pl.BlockSpec((TM, D), lambda i: (i, 0)),
        out_shape=jax.ShapeDtypeStruct((S, D), A_x.dtype),
        scratch_shapes=[
            pltpu.VMEM((NBLK, NG, QB // R, 128), pk),
            pltpu.VMEM((NBLK, 768 // R, QB), pk),
            pltpu.VMEM((NQ, NG, QB // R, 128), pk),
            pltpu.VMEM((D, D), jnp.bfloat16),
            pltpu.VMEM((TM // R, D), pk),
            pltpu.VMEM((TM // R, F), pk),
            pltpu.VMEM((TM, 128), jnp.float32),
            pltpu.VMEM((S // TM, TM, D), jnp.bfloat16),
            pltpu.VMEM((D, 2 * D), jnp.bfloat16),
            pltpu.VMEM((D, D), jnp.bfloat16),
            pltpu.VMEM((D, D), jnp.bfloat16),
            pltpu.VMEM((D, F), jnp.bfloat16),
            pltpu.VMEM((F, D), jnp.bfloat16),
            pltpu.VMEM((D,), jnp.bfloat16),
            pltpu.SemaphoreType.DMA((6 + S // TM,)),
        ],
        compiler_params=pltpu.CompilerParams(
            dimension_semantics=("arbitrary",), vmem_limit_bytes=100 * 2**20, flags=flags),
    )(x, A_wqkv, A_wo, B_w1, B_w2, gate_w)
    return out.reshape(1, S, D)
```

```python
import math

import jax
import jax.numpy as jnp
from jax import lax
import jax.experimental.pallas as pl
import jax.experimental.pallas.tpu as pltpu

S, D, H, DH, F = 2048, 640, 32, 20, 1536
QB = 128
TM = 512
NQ = TM // QB
NS = S // TM
NG = H // 4
SKEW = 4
NEG = -1e30
ONE = 0x3F80
NT = (((1,), (1,)), ((), ()))


def _window(g):
    return 64 * ((80 * g) // 64)


def _flag_lanes(g):
    return (80 * g + 112) % 128, (80 * g + 80) % 128


def _kernel(x_hbm, wqkv_hbm, wo_hbm, w1_hbm, w2_hbm, gw_hbm, o_ref,
            klo_ref, khi_ref, k2_ref, vt_ref, qt_ref, wqvt_ref, co_ref, ch_ref, g_ref,
            xs_ref, wq_ref, wk_ref, wv_ref, wo_ref, w1_ref, w2_ref, gw_ref, sems):
    f32, bf16, u32 = jnp.float32, jnp.bfloat16, jnp.uint32
    unpack = lambda v: pltpu.bitcast(v, bf16)
    pack = lambda v: pltpu.bitcast(v, u32)
    i = pl.program_id(0)
    lane = lax.broadcasted_iota(jnp.int32, (QB // 2, 128), 1)

    def x_copy(c):
        return pltpu.make_async_copy(x_hbm.at[pl.ds(c * TM, TM)], xs_ref.at[c], sems.at[7 + c])
    wq_copy = pltpu.make_async_copy(wqkv_hbm.at[:, pl.ds(0, D)], wq_ref, sems.at[0])
    wk_copy = pltpu.make_async_copy(wqkv_hbm.at[:, pl.ds(D, D)], wk_ref, sems.at[6])
    wv_copy = pltpu.make_async_copy(wqkv_hbm.at[:, pl.ds(2 * D, D)], wv_ref, sems.at[1])
    gw_copy = pltpu.make_async_copy(gw_hbm, gw_ref, sems.at[2])
    w1_copy = pltpu.make_async_copy(w1_hbm, w1_ref, sems.at[3])
    w2_copy = pltpu.make_async_copy(w2_hbm, w2_ref, sems.at[4])
    wo_copy = pltpu.make_async_copy(wo_hbm, wo_ref, sems.at[5])

    @pl.when(i == 0)
    def _():
        for cp in (wq_copy, wv_copy, x_copy(0), gw_copy, wk_copy, w1_copy, wo_copy, w2_copy):
            cp.start()
        for c in range(1, NS):
            x_copy(c).start()
        for g in range(NG):
            fa, fb = _flag_lanes(g)
            pad = pack(jnp.where((lane == fa) | (lane == fb), NEG, 0.0).astype(bf16))
            for b in range(2):
                klo_ref[b, g] = pad
                khi_ref[b, g] = pad
        vt_ref[0:2] = jnp.zeros((2, 384, QB), u32)
        for part, (cp, ref) in enumerate(((wq_copy, wq_ref), (wv_copy, wv_ref))):
            cp.wait()
            for t in range(5):
                w = ref[:, 128 * t:128 * (t + 1)].astype(f32)
                r0 = part * D + 128 * t
                wqvt_ref[r0:r0 + 128, :] = w.T.astype(bf16)
        gw_copy.wait()
        wk_copy.wait()

    x_copy(i).wait()
    x = xs_ref[i]

    qv = lax.dot_general(wqvt_ref[...], x, NT, preferred_element_type=f32)
    qt, vt = qv[0:D], qv[D:]
    qtp = pack((qt * ((DH ** -0.5) * math.log2(math.e))).astype(bf16))
    ones = jnp.ones((8, TM), f32)
    parts = []
    for p in range(H // 2):
        parts += [vt[40 * p:40 * p + 24], ones, vt[40 * p + 24:40 * p + 40]]
    vtp = pack(jnp.concatenate(parts, axis=0).astype(bf16))
    for j in range(NQ):
        qt_ref[j] = qtp[:, j * QB:(j + 1) * QB]
        vt_ref[2 + j] = vtp[:, j * QB:(j + 1) * QB]

    for j in range(NQ):
        kj = jnp.dot(x[j * QB:(j + 1) * QB], wk_ref[...], preferred_element_type=f32).astype(bf16)
        slabs = [pack(kj[:, 128 * t:128 * (t + 1)]) for t in range(5)]
        for g in range(NG):
            w0 = _window(g)
            t = w0 // 128
            win = slabs[t] if w0 % 128 == 0 else jnp.where(lane < 64, slabs[t + 1], slabs[t])
            fa, fb = _flag_lanes(g)
            k2_ref[j, g] = pltpu.roll(win[QB // 4:], 64, 1)
            win = jnp.where((lane == fa) | (lane == fb), jnp.uint32(0), win)
            klo_ref[2 + j, g] = win[0:QB // 4]
            khi_ref[2 + j, g] = win[QB // 4:]

    logit = jnp.sum(x.astype(f32) * gw_ref[...].astype(f32)[None, :], axis=1, keepdims=True)
    g_ref[...] = jnp.broadcast_to(jax.nn.sigmoid(logit), (TM, 128))

    row = lax.broadcasted_iota(jnp.int32, (QB, QB), 0)
    col = lax.broadcasted_iota(jnp.int32, (QB, QB), 1)
    tri = row > col
    sub = lax.broadcasted_iota(jnp.int32, (8, QB), 0)
    lane8 = lax.broadcasted_iota(jnp.int32, (8, QB), 1)
    lane32 = lax.broadcasted_iota(jnp.int32, (QB // 4, QB), 1)
    zero8 = lambda: jnp.zeros((8, QB), u32)

    def q_pieces(j, g, t, flag_lane):
        w0 = _window(g)
        f_lo, f_hi = DH * (4 * g + t), DH * (4 * g + t + 1)
        fl = flag_lane // 2
        feats, flags = [], []
        for v in range(8):
            fbase = w0 + ((16 * v - w0) % 128)
            lo = max(f_lo, fbase) - fbase
            hi = min(f_hi, fbase + 16) - fbase
            if hi > lo:
                src = qt_ref[j, fbase // 2:fbase // 2 + 8, :]
                if lo == 0 and hi == 16:
                    feats.append(src)
                else:
                    feats.append(jnp.where((sub >= lo // 2) & (sub < hi // 2), src, jnp.uint32(0)))
            else:
                feats.append(None)
            flags.append(sub == fl - 8 * v if 8 * v <= fl < 8 * v + 8 else None)
        return feats, flags

    def q_tile(feats, flags):
        pieces = []
        for v in range(8):
            p = feats[v]
            if flags[v] is not None:
                p = jnp.where(flags[v], jnp.uint32(ONE), zero8() if p is None else p)
            pieces.append(zero8() if p is None else p)
        return unpack(jnp.concatenate(pieces, axis=0))

    def q_tile_merged(feats, flags):
        left = lane8 < 64
        pieces = []
        for v in range(8):
            a = feats[v]
            if flags[v] is not None:
                a = jnp.where(flags[v], jnp.uint32(ONE), zero8() if a is None else a)
            b = feats[(v - 4) % 8]
            if a is None and b is None:
                pieces.append(zero8())
            elif b is None:
                pieces.append(jnp.where(left, a, jnp.uint32(0)))
            elif a is None:
                pieces.append(jnp.where(left, jnp.uint32(0), b))
            else:
                pieces.append(jnp.where(left, a, b))
        return unpack(jnp.concatenate(pieces, axis=0))

    def scores(j, g):
        fa, fb = _flag_lanes(g)
        pcs = [q_pieces(j, g, t, (fa, fb)[t // 2]) for t in range(4)]
        qm = jnp.concatenate([q_tile(*pcs[t]) for t in range(4)], axis=1)
        kf_lo, kf_hi = klo_ref[j, g], khi_ref[j, g]
        km_lo, km_hi = klo_ref[j + 1, g], khi_ref[j + 1, g]
        kl_lo = klo_ref[j + 2, g]
        k2 = k2_ref[j, g]
        merged = []
        for p in range(2):
            lo = (80 * g + 40 * p + 64) % 128
            hi = lo + 40
            m = (lane32 >= lo) & (lane32 < hi)
            if hi > 128:
                m = m | (lane32 < hi - 128)
            lhs = unpack(jnp.where(m, k2, kf_lo))
            w = jnp.concatenate([q_tile_merged(*pcs[2 * p + t]) for t in range(2)], axis=1)
            merged.append(jnp.dot(lhs, w, preferred_element_type=f32))
        ks = unpack(jnp.concatenate([kf_hi, kl_lo, km_lo, km_hi], axis=0))
        s = jnp.dot(ks, qm, preferred_element_type=f32)
        out = []
        for t in range(4):
            st = s[:, 128 * t:128 * (t + 1)]
            mg = merged[t // 2][:, 128 * (t % 2):128 * (t % 2 + 1)]
            comb = jnp.concatenate([jnp.where(tri[0:64], mg, st[64:128]),
                                    jnp.where(tri[64:], st[0:64], mg)], axis=0)
            out.append((comb, st[128:]))
        res = []
        for comb, mid in out:
            m = jnp.maximum(jnp.max(comb, axis=0, keepdims=True), jnp.max(mid, axis=0, keepdims=True))
            res.append((m, comb, mid))
        return res

    def head_out(j, g, t, state):
        m, comb, mid = state
        h = 4 * g + t
        pc = jnp.exp2(comb - m)
        p1 = jnp.exp2(mid - m)
        p0 = jnp.where(tri, pc, 0.0)
        p2 = jnp.where(tri, 0.0, pc)
        ra = (48 * (h // 2) + (0 if h % 2 == 0 else 32)) // 2
        rb = (48 * (h // 2) + 16) // 2
        p = jnp.concatenate([p0, p1, p2], axis=0).astype(bf16)
        lhs = jnp.concatenate(
            [jnp.concatenate([unpack(vt_ref[j + c, ra:ra + 8, :]), unpack(vt_ref[j + c, rb:rb + 8, :])], axis=0)
             for c in range(3)], axis=1)
        r = jnp.dot(lhs, p, preferred_element_type=f32)
        inv = 1.0 / r[24:32]
        return r[0:8] * inv, r[8:16] * inv, r[16:24] * inv

    def pair_rows(e, o):
        return [e[0], e[1], jnp.where(sub < 4, e[2], o[2]), o[0], o[1]]

    def finish_block(j, rows):
        ot = jnp.concatenate(rows, axis=0)
        gg = g_ref[j * QB:(j + 1) * QB, :]
        for t in range(5):
            o_t = ot[128 * t:128 * (t + 1)].T
            co_ref[j * QB // 2:(j + 1) * QB // 2, 128 * t:128 * (t + 1)] = pack((o_t * gg).astype(bf16))

    units = [(j, g) for j in range(NQ) for g in range(NG)]
    pending = {u: scores(*units[u]) for u in range(SKEW)}
    rows = []
    for u, (j, g) in enumerate(units):
        state = pending.pop(u)
        res = [head_out(j, g, t, state[t]) for t in range(2)]
        if u + SKEW < len(units):
            pending[u + SKEW] = scores(*units[u + SKEW])
        res += [head_out(j, g, t, state[t]) for t in range(2, 4)]
        rows += pair_rows(res[0], res[1]) + pair_rows(res[2], res[3])
        if g == NG - 1:
            finish_block(j, rows)
            rows = []

    for b in range(2):
        klo_ref[b] = klo_ref[NQ + b]
        khi_ref[b] = khi_ref[NQ + b]
        vt_ref[b] = vt_ref[NQ + b]

    @pl.when(i == 0)
    def _():
        wo_copy.wait()
        w1_copy.wait()
        w2_copy.wait()

    g1 = 1.0 - g_ref[:, 0:1]
    u_ = 0.5 * jnp.dot(x, w1_ref[...], preferred_element_type=f32)
    ch_ref[...] = pack(((u_ + u_ * jnp.tanh(u_)) * g1).astype(bf16))
    out = jnp.dot(unpack(co_ref[...]), wo_ref[...], preferred_element_type=f32)
    out = out + jnp.dot(unpack(ch_ref[...]), w2_ref[...], preferred_element_type=f32)
    o_ref[...] = out.astype(o_ref.dtype)


@jax.jit
def pallas_gated_mix__sliding_block__dense_activation_silu__prompt_kernel(
    A_x: jax.Array,
    A_wqkv: jax.Array,
    A_wo: jax.Array,
    B_x: jax.Array,
    B_w1: jax.Array,
    B_w2: jax.Array,
    gate_w: jax.Array,
):
    del B_x
    assert A_x.shape == (1, S, D) and B_w1.shape == (D, F)
    u32, bf16 = jnp.uint32, jnp.bfloat16
    hbm = pl.BlockSpec(memory_space=pl.ANY)
    out = pl.pallas_call(
        _kernel,
        grid=(NS,),
        in_specs=[hbm] * 6,
        out_specs=pl.BlockSpec((TM, D), lambda i: (i, 0)),
        out_shape=jax.ShapeDtypeStruct((S, D), A_x.dtype),
        scratch_shapes=[
            pltpu.VMEM((NQ + 2, NG, QB // 4, 128), u32),
            pltpu.VMEM((NQ + 2, NG, QB // 4, 128), u32),
            pltpu.VMEM((NQ, NG, QB // 4, 128), u32),
            pltpu.VMEM((NQ + 2, 384, QB), u32),
            pltpu.VMEM((NQ, D // 2, QB), u32),
            pltpu.VMEM((2 * D, D), bf16),
            pltpu.VMEM((TM // 2, D), u32),
            pltpu.VMEM((TM // 2, F), u32),
            pltpu.VMEM((TM, 128), jnp.float32),
            pltpu.VMEM((NS, TM, D), bf16),
            pltpu.VMEM((D, D), bf16),
            pltpu.VMEM((D, D), bf16),
            pltpu.VMEM((D, D), bf16),
            pltpu.VMEM((D, D), bf16),
            pltpu.VMEM((D, F), bf16),
            pltpu.VMEM((F, D), bf16),
            pltpu.VMEM((D,), bf16),
            pltpu.SemaphoreType.DMA((7 + NS,)),
        ],
        compiler_params=pltpu.CompilerParams(
            dimension_semantics=("arbitrary",), vmem_limit_bytes=100 * 2**20),
    )(A_x.reshape(S, D), A_wqkv, A_wo, B_w1, B_w2, gate_w)
    return out.reshape(1, S, D)
```
